```python
import jax
import jax.numpy as jnp

def _softmax(x, axis=-1):
    return jax.nn.softmax(x, axis=axis)

def _gelu(x):
    return jax.nn.gelu(x, approximate=True)

def _silu(x):
    return jax.nn.silu(x)

def _sigmoid(x):
    return jax.nn.sigmoid(x)

def _layernorm(x, axis=-1, eps=1e-05):
    m = jnp.mean(x, axis=axis, keepdims=True)
    v = jnp.var(x, axis=axis, keepdims=True)
    return (x - m) / jnp.sqrt(v + eps)

def _scatter_add(tgt, idx, src, axis=0):
    return tgt.at[idx].add(src)

def _segment_sum(src, seg, n):
    return jax.ops.segment_sum(src, seg, n)

class _Rng:

    def __init__(self, key):
        self._k = key

    def _next(self):
        self._k, sub = jax.random.split(self._k)
        return sub

    def normal(self, shape):
        return jax.random.normal(self._next(), shape, dtype=jnp.bfloat16)

    def randint(self, lo, hi, shape):
        return jax.random.randint(self._next(), shape, lo, hi, dtype=jnp.int32)

    def uniform(self, shape, lo=0.0, hi=1.0):
        return jax.random.uniform(self._next(), shape, jnp.bfloat16, lo, hi)

    def permutation(self, n):
        return jax.random.permutation(self._next(), n)
kernel_name = 'standalone__dilated_atrous__vision'

def setup_inputs():
    _rng = _Rng(jax.random.key(int.from_bytes(__import__("os").urandom(4), "little")))
    _w = lambda a: (lambda t: t.astype(jnp.bfloat16) if jnp.issubdtype(t.dtype, jnp.floating) else t)(jnp.asarray(a))
    H = W = 384
    C = 384
    k = 1
    return {'x': _w((lambda *s: _rng.normal(s) * 0.05)(1, H, W, C)), 'w': _w((lambda *s: _rng.normal(s) * 0.05)(k, k, C, C) * (1.0 / (k * C ** 0.5)))}

def reference(x, w):
    B, H, W, C = x.shape
    k = 1
    rate = 2
    pad = (k - 1) * rate // 2
    xp = jnp.pad(x, ((0, 0), (pad, pad), (pad, pad), (0, 0)))
    out = jnp.zeros_like(x)
    for i in range(k):
        for j in range(k):
            tap = xp[:, i * rate:i * rate + H, j * rate:j * rate + W, :].copy()
            out = out + jnp.einsum('bhwc,co->bhwo', tap, w[i, j])
    return out
```

```python
import functools

import jax
import jax.numpy as jnp
import jax.experimental.pallas as pl
import jax.experimental.pallas.tpu as pltpu

_BM = 2048
_STREAMS = 8
_PIECE = 16
_RD_BLOCKS = 2
_LEAD = 6


def _kernel(x_hbm, w_ref, o_hbm, buf, rsem, wsem):
    n, bm, _ = buf.shape
    k, p, rb = _STREAMS, _PIECE, _RD_BLOCKS
    nc = bm // p
    nr = n // rb
    n1 = n // 2 + _LEAD
    steps = n // 2
    wps = (n // k) * nc // steps
    for t in range(steps):
        assert (((t + 1) * wps - 1) // nc + 1) * k <= min(n, n1 + max(t - 1, 0))

    def read(j):
        sl = pl.ds(j * rb, rb)
        return pltpu.make_async_copy(x_hbm.at[sl], buf.at[sl], rsem.at[j])

    def write(i, slot):
        gs = pl.ds((i // nc) * k, k)
        cs = pl.ds(pl.multiple_of((i % nc) * p, p), p)
        return pltpu.make_async_copy(buf.at[gs, cs], o_hbm.at[gs, cs], wsem.at[slot])

    def compute(i):
        buf[i] = jnp.dot(
            buf[i], w_ref[...], preferred_element_type=jnp.float32
        ).astype(buf.dtype)

    def start_writes(t):
        for u in range(wps):
            write(t * wps + u, t % 2).start()

    def wait_writes(t):
        for u in range(wps):
            write(t * wps + u, t % 2).wait()

    for j in range(nr):
        read(j).start()

    def read_step(i, _):
        @pl.when(i % rb == 0)
        def _():
            read(i // rb).wait()

        compute(i)

    jax.lax.fori_loop(0, n1, read_step, None)
    for j in range(pl.cdiv(n1, rb), nr):
        read(j).wait()

    start_writes(0)

    def write_step(t, _):
        start_writes(t + 1)

        @pl.when(n1 + t < n)
        def _():
            compute(n1 + t)

        wait_writes(t)

    jax.lax.fori_loop(0, steps - 1, write_step, None)
    wait_writes(steps - 1)


@jax.jit
def pallas_standalone__dilated_atrous__vision_kernel(
    x: jax.Array,
    w: jax.Array,
):
    B, H, W, C = x.shape
    assert w.shape == (1, 1, C, C)
    n = B * H * W // _BM
    out = pl.pallas_call(
        _kernel,
        in_specs=[
            pl.BlockSpec(memory_space=pl.ANY),
            pl.BlockSpec(memory_space=pltpu.VMEM),
        ],
        out_specs=pl.BlockSpec(memory_space=pl.ANY),
        out_shape=jax.ShapeDtypeStruct((n, _BM, C), x.dtype),
        scratch_shapes=[
            pltpu.VMEM((n, _BM, C), x.dtype),
            pltpu.SemaphoreType.DMA((n // _RD_BLOCKS,)),
            pltpu.SemaphoreType.DMA((2,)),
        ],
        compiler_params=pltpu.CompilerParams(vmem_limit_bytes=126 * 1024 * 1024),
    )(x.reshape(n, _BM, C), w.reshape(C, C))
    return out.reshape(B, H, W, C)
```

```python
import jax
import jax.numpy as jnp
import jax.experimental.pallas as pl
import jax.experimental.pallas.tpu as pltpu

_BM = 2048
_RD_COMPUTE = 40
_SEG = 128
_LAG = 3
_HI_STREAMS = 2
_HI_ROWS = 16
_LO_BLOCKS = 2
_TAIL = 512
_WR_STREAMS = 6
_WR_ROWS = 16
_WR_STEP = 1024
_WR_FIRST = 24
_WR_PER_STEP = 20


def _kernel(x_hbm, w_hbm, o_hbm, buf, wbuf, lo_sem, sem):
    n, bm, c = buf.shape
    hi_sem, wr_sem, w_sem, tail_sem = (sem.at[i] for i in range(4))

    n_rd = _RD_COMPUTE
    segs = (bm // _SEG) * (c // 128)
    n_hi = n_rd * segs * _HI_STREAMS * _HI_ROWS // bm
    n_lo = n - n_hi
    n_lo_dma = n_lo // _LO_BLOCKS
    hi_per_group = bm // _HI_ROWS
    wr_per_group = bm // _WR_ROWS
    n_wr = (n // _WR_STREAMS) * wr_per_group
    steps_per_block = bm // _WR_STEP
    steps = (n - n_rd) * steps_per_block
    assert n_hi * bm == n_rd * segs * _HI_STREAMS * _HI_ROWS
    assert n_hi % _HI_STREAMS == 0 and n_lo % _LO_BLOCKS == 0
    assert n % _WR_STREAMS == 0 and n_rd <= n_lo - _LO_BLOCKS
    assert _LAG >= c // 128
    for u in range(-1, steps):
        done = n_rd + max(u, 0) // steps_per_block
        queued = _WR_FIRST + (u + 1) * _WR_PER_STEP
        assert queued <= wr_per_group * (done // _WR_STREAMS)

    def read(blocks, rows, s):
        return pltpu.make_async_copy(x_hbm.at[blocks, rows], buf.at[blocks, rows], s)

    def read_lo(g):
        return read(pl.ds(g * _LO_BLOCKS, _LO_BLOCKS), pl.ds(0, bm), lo_sem.at[g])

    def read_hi(j):
        blocks = pl.ds(n_lo + (j // hi_per_group) * _HI_STREAMS, _HI_STREAMS)
        row0 = pl.multiple_of((j % hi_per_group) * _HI_ROWS, _HI_ROWS)
        return read(blocks, pl.ds(row0, _HI_ROWS), hi_sem)

    def read_last():
        blocks = pl.ds(n_lo - _LO_BLOCKS, _LO_BLOCKS)
        return (
            read(blocks, pl.ds(0, bm - _TAIL), lo_sem.at[n_lo_dma - 1]),
            read(blocks, pl.ds(bm - _TAIL, _TAIL), tail_sem),
        )

    def start_write(i, _):
        blocks = pl.ds((i // wr_per_group) * _WR_STREAMS, _WR_STREAMS)
        row0 = pl.multiple_of((i % wr_per_group) * _WR_ROWS, _WR_ROWS)
        rows = pl.ds(row0, _WR_ROWS)
        pltpu.make_async_copy(
            buf.at[blocks, rows], o_hbm.at[blocks, rows], wr_sem
        ).start()

    def matmul(a, b):
        return jnp.dot(a, b, preferred_element_type=jnp.float32).astype(buf.dtype)

    w_copy = pltpu.make_async_copy(w_hbm, wbuf, w_sem)
    w_copy.start()

    def start_lo(g, _):
        head, tail = read_last()
        pl.when(g < n_lo_dma - 1)(lambda: read_lo(g).start(priority=1))
        pl.when(g == n_lo_dma - 1)(lambda: head.start(priority=1))
        pl.when(g == n_lo_dma)(lambda: tail.start(priority=1))

    jax.lax.fori_loop(0, n_lo_dma + 1, start_lo, None)
    w_copy.wait()

    def read_step(i, _):
        pl.when(i % _LO_BLOCKS == 0)(lambda: read_lo(i // _LO_BLOCKS).wait())
        pending = []
        for q in range(segs):
            rows = pl.ds(q // (c // 128) * _SEG, _SEG)
            cols = pl.ds(q % (c // 128) * 128, 128)
            if len(pending) == _LAG:
                r, cl, y = pending.pop(0)
                buf[i, r, cl] = y
            read_hi(i * segs + q).start()
            pending.append((rows, cols, matmul(buf[i, rows], wbuf[:, cols])))
        for r, cl, y in pending:
            buf[i, r, cl] = y

    jax.lax.fori_loop(0, n_rd, read_step, None)
    for g in range(pl.cdiv(n_rd, _LO_BLOCKS), n_lo_dma - 1):
        read_lo(g).wait()
    read(pl.ds(n_lo, n_hi), pl.ds(0, bm), hi_sem).wait()
    head, tail = read_last()
    head.wait()

    jax.lax.fori_loop(0, _WR_FIRST, start_write, None)
    tail.wait()

    def write_step(u, _):
        first = _WR_FIRST + u * _WR_PER_STEP
        jax.lax.fori_loop(first, first + _WR_PER_STEP, start_write, None)
        i = n_rd + u // steps_per_block
        rows = pl.ds(pl.multiple_of((u % steps_per_block) * _WR_STEP, _WR_STEP), _WR_STEP)
        buf[i, rows] = matmul(buf[i, rows], wbuf[...])

    jax.lax.fori_loop(0, steps, write_step, None)
    jax.lax.fori_loop(_WR_FIRST + steps * _WR_PER_STEP, n_wr, start_write, None)
    pltpu.make_async_copy(buf, o_hbm, wr_sem).wait()


@jax.jit
def pallas_standalone__dilated_atrous__vision_kernel(
    x: jax.Array,
    w: jax.Array,
):
    B, H, W, C = x.shape
    assert w.shape == (1, 1, C, C)
    n = B * H * W // _BM
    out = pl.pallas_call(
        _kernel,
        in_specs=[
            pl.BlockSpec(memory_space=pl.ANY),
            pl.BlockSpec(memory_space=pl.ANY),
        ],
        out_specs=pl.BlockSpec(memory_space=pl.ANY),
        out_shape=jax.ShapeDtypeStruct((n, _BM, C), x.dtype),
        scratch_shapes=[
            pltpu.VMEM((n, _BM, C), x.dtype),
            pltpu.VMEM((C, C), w.dtype),
            pltpu.SemaphoreType.DMA((n // _LO_BLOCKS,)),
            pltpu.SemaphoreType.DMA((4,)),
        ],
        compiler_params=pltpu.CompilerParams(
            vmem_limit_bytes=126 * 1024 * 1024,
            disable_bounds_checks=True,
        ),
    )(x.reshape(n, _BM, C), w.reshape(C, C))
    return out.reshape(B, H, W, C)
```

```python
import jax
import jax.numpy as jnp
import jax.experimental.pallas as pl
import jax.experimental.pallas.tpu as pltpu

_LANES = 128
_BM = 2048
_STREAMS = 6
_PIECE = 16
_RD_BLOCKS = 40
_SEG = 128
_LO_BLOCKS = 2
_TAIL = 512
_WR_ROWS = 1024
_WR_FIRST = 24
_WR_PER_STEP = 20


def _kernel(x_hbm, w_hbm, o_hbm, buf, wbuf, lo_sem, sem):
    n, bm, c = buf.shape
    hi_sem, wr_sem, w_sem, tail_sem = (sem.at[i] for i in range(4))

    col_tiles = c // _LANES
    segs = bm // _SEG
    pieces = bm // _PIECE
    n_hi = _RD_BLOCKS * segs // pieces * _STREAMS
    n_lo = n - n_hi
    n_lo_dma = n_lo // _LO_BLOCKS
    n_wr = n // _STREAMS * pieces
    steps_per_block = bm // _WR_ROWS
    steps = (n - _RD_BLOCKS) * steps_per_block
    assert _RD_BLOCKS * segs % pieces == 0 and n % _STREAMS == 0
    assert n_lo % _LO_BLOCKS == 0 and _RD_BLOCKS <= n_lo - _LO_BLOCKS
    for u in range(-1, steps):
        done = _RD_BLOCKS + max(u, 0) // steps_per_block
        assert _WR_FIRST + (u + 1) * _WR_PER_STEP <= pieces * (done // _STREAMS)

    def piece(block0, j):
        blocks = pl.ds(block0 + j // pieces * _STREAMS, _STREAMS)
        rows = pl.ds(pl.multiple_of(j % pieces * _PIECE, _PIECE), _PIECE)
        return blocks, rows

    def read(window, s):
        return pltpu.make_async_copy(x_hbm.at[window], buf.at[window], s)

    def read_lo(g):
        return read((pl.ds(g * _LO_BLOCKS, _LO_BLOCKS),), lo_sem.at[g])

    def read_lo_last():
        blocks = pl.ds(n_lo - _LO_BLOCKS, _LO_BLOCKS)
        return (
            read((blocks, pl.ds(0, bm - _TAIL)), lo_sem.at[n_lo_dma - 1]),
            read((blocks, pl.ds(bm - _TAIL, _TAIL)), tail_sem),
        )

    def start_write(j, _):
        window = piece(0, j)
        pltpu.make_async_copy(buf.at[window], o_hbm.at[window], wr_sem).start()

    def wait_total(ref, s):
        pltpu.make_async_copy(ref, ref, s).wait()

    def matmul(a, b):
        return jnp.dot(a, b, preferred_element_type=jnp.float32).astype(buf.dtype)

    w_copy = pltpu.make_async_copy(w_hbm, wbuf, w_sem)
    w_copy.start()

    def start_lo(g, _):
        head, tail = read_lo_last()
        pl.when(g < n_lo_dma - 1)(lambda: read_lo(g).start(priority=1))
        pl.when(g == n_lo_dma - 1)(lambda: head.start(priority=1))
        pl.when(g == n_lo_dma)(lambda: tail.start(priority=1))

    jax.lax.fori_loop(0, n_lo_dma + 1, start_lo, None)
    w_copy.wait()

    def read_step(i, _):
        pl.when(i % _LO_BLOCKS == 0)(lambda: read_lo(i // _LO_BLOCKS).wait())
        pending = []
        for s in range(segs):
            rows = pl.ds(s * _SEG, _SEG)
            for t in range(col_tiles):
                cols = pl.ds(t * _LANES, _LANES)
                if len(pending) == col_tiles:
                    r, cl, y = pending.pop(0)
                    buf[i, r, cl] = y
                if t == 0:
                    read(piece(n_lo, i * segs + s), hi_sem).start()
                pending.append((rows, cols, matmul(buf[i, rows], wbuf[:, cols])))
        for r, cl, y in pending:
            buf[i, r, cl] = y

    jax.lax.fori_loop(0, _RD_BLOCKS, read_step, None)
    for g in range(pl.cdiv(_RD_BLOCKS, _LO_BLOCKS), n_lo_dma - 1):
        read_lo(g).wait()
    wait_total(buf.at[pl.ds(n_lo, n_hi)], hi_sem)
    head, tail = read_lo_last()
    head.wait()

    jax.lax.fori_loop(0, _WR_FIRST, start_write, None)
    tail.wait()

    def write_step(u, _):
        first = _WR_FIRST + u * _WR_PER_STEP
        jax.lax.fori_loop(first, first + _WR_PER_STEP, start_write, None)
        i = _RD_BLOCKS + u // steps_per_block
        row0 = pl.multiple_of(u % steps_per_block * _WR_ROWS, _WR_ROWS)
        rows = pl.ds(row0, _WR_ROWS)
        buf[i, rows] = matmul(buf[i, rows], wbuf[...])

    jax.lax.fori_loop(0, steps, write_step, None)
    jax.lax.fori_loop(_WR_FIRST + steps * _WR_PER_STEP, n_wr, start_write, None)
    wait_total(buf, wr_sem)


@jax.jit
def pallas_standalone__dilated_atrous__vision_kernel(
    x: jax.Array,
    w: jax.Array,
):
    B, H, W, C = x.shape
    assert w.shape == (1, 1, C, C)
    n = B * H * W // _BM
    out = pl.pallas_call(
        _kernel,
        in_specs=[
            pl.BlockSpec(memory_space=pl.ANY),
            pl.BlockSpec(memory_space=pl.ANY),
        ],
        out_specs=pl.BlockSpec(memory_space=pl.ANY),
        out_shape=jax.ShapeDtypeStruct((n, _BM, C), x.dtype),
        scratch_shapes=[
            pltpu.VMEM((n, _BM, C), x.dtype),
            pltpu.VMEM((C, C), w.dtype),
            pltpu.SemaphoreType.DMA((n // _LO_BLOCKS,)),
            pltpu.SemaphoreType.DMA((4,)),
        ],
        compiler_params=pltpu.CompilerParams(
            vmem_limit_bytes=116 * 1024 * 1024,
            disable_bounds_checks=True,
        ),
    )(x.reshape(n, _BM, C), w.reshape(C, C))
    return out.reshape(B, H, W, C)
```
